```python
import jax
import jax.numpy as jnp

def _softmax(x, axis=-1):
    return jax.nn.softmax(x, axis=axis)

def _gelu(x):
    return jax.nn.gelu(x, approximate=True)

def _silu(x):
    return jax.nn.silu(x)

def _sigmoid(x):
    return jax.nn.sigmoid(x)

def _layernorm(x, axis=-1, eps=1e-05):
    m = jnp.mean(x, axis=axis, keepdims=True)
    v = jnp.var(x, axis=axis, keepdims=True)
    return (x - m) / jnp.sqrt(v + eps)

def _scatter_add(tgt, idx, src, axis=0):
    return tgt.at[idx].add(src)

def _segment_sum(src, seg, n):
    return jax.ops.segment_sum(src, seg, n)

class _Rng:

    def __init__(self, key):
        self._k = key

    def _next(self):
        self._k, sub = jax.random.split(self._k)
        return sub

    def normal(self, shape):
        return jax.random.normal(self._next(), shape, dtype=jnp.bfloat16)

    def randint(self, lo, hi, shape):
        return jax.random.randint(self._next(), shape, lo, hi, dtype=jnp.int32)

    def uniform(self, shape, lo=0.0, hi=1.0):
        return jax.random.uniform(self._next(), shape, jnp.bfloat16, lo, hi)

    def permutation(self, n):
        return jax.random.permutation(self._next(), n)
kernel_name = 'adaLN_cond__sliding_block_cached__moe_arch_mod__prompt'

def setup_inputs():
    _rng = _Rng(jax.random.key(int.from_bytes(__import__("os").urandom(4), "little")))
    _w = lambda a: (lambda t: t.astype(jnp.bfloat16) if jnp.issubdtype(t.dtype, jnp.floating) else t)(jnp.asarray(a))

    def _A_setup():
        B, Sq, D = (1, 2048, 1024)
        Hq, Hkv, Sk, Dh = (32, 4, 2048, 128)
        assert Hq % Hkv == 0, (Hq, Hkv)
        return {'x': _w((lambda *s: _rng.normal(s) * 0.05)(B, Sq, D)), 'k_cache': _w((lambda *s: _rng.normal(s) * 0.05)(B, Hkv, Sk, Dh)), 'v_cache': _w((lambda *s: _rng.normal(s) * 0.05)(B, Hkv, Sk, Dh)), 'wq': _w((lambda *s: _rng.normal(s) * 0.05)(D, Hq * Dh) * D ** (-0.5)), 'wo': _w((lambda *s: _rng.normal(s) * 0.05)(Hq * Dh, D) * (Hq * Dh) ** (-0.5))}
    _A_in = _A_setup()

    def _B_setup():
        B, S, D, F, C = (1, 2048, 1024, 3584, 1)
        return {'x': _w((lambda *s: _rng.normal(s) * 0.05)(B, S, D)), 'w_r': _w((lambda *s: _rng.normal(s) * 0.05)(D)), 'w_gate': _w((lambda *s: _rng.normal(s) * 0.05)(D, F)), 'w_up': _w((lambda *s: _rng.normal(s) * 0.05)(D, F)), 'w_down': _w((lambda *s: _rng.normal(s) * 0.05)(F, D))}
    _B_in = _B_setup()
    return {'A_x': _A_in['x'], 'A_k_cache': _A_in['k_cache'], 'A_v_cache': _A_in['v_cache'], 'A_wq': _A_in['wq'], 'A_wo': _A_in['wo'], 'B_x': _B_in['x'], 'B_w_r': _B_in['w_r'], 'B_w_gate': _B_in['w_gate'], 'B_w_up': _B_in['w_up'], 'B_w_down': _B_in['w_down'], 'c': _w((lambda *s: _rng.normal(s) * 0.05)(1, 1024)), 'w_mod': _w((lambda *s: _rng.normal(s) * 0.05)(1024, 6 * 1024) * 1024 ** (-0.5))}

def reference(A_x, A_k_cache, A_v_cache, A_wq, A_wo, B_x, B_w_r, B_w_gate, B_w_up, B_w_down, c, w_mod):

    def _A_ref(x, k_cache, v_cache, wq, wo):
        B, Sq, D = x.shape
        Hq, Dh = (32, 128)
        Hkv, Sk = (k_cache.shape[1], k_cache.shape[2])
        W = min(4096, max(256, Sk // 4))
        rep = Hq // Hkv
        q = (lambda x, *d: x.transpose(*d))((x @ wq).reshape(B, Sq, Hq, Dh), 0, 2, 1, 3)
        k = jnp.repeat(k_cache[:, :, Sk - W:, :], rep, axis=1)
        v = jnp.repeat(v_cache[:, :, Sk - W:, :], rep, axis=1)
        scores = jnp.einsum('bhqd,bhkd->bhqk', q, k) * Dh ** (-0.5)
        p = _softmax(scores, axis=-1)
        o = jnp.einsum('bhqk,bhkd->bhqd', p, v)
        return (lambda x, *d: x.transpose(*d))(o, 0, 2, 1, 3).reshape(B, Sq, Hq * Dh) @ wo

    def _B_ref(x, w_r, w_gate, w_up, w_down):
        B, S, D = x.shape
        C = 1
        r = x @ w_r
        idx = jnp.argsort(-r, axis=-1)[:, :C]
        idx_e = jnp.repeat(idx.reshape(B, C, 1), D, axis=2)
        x_sel = jnp.take_along_axis(x, idx_e, axis=1)
        g = _silu(x_sel @ w_gate)
        u = x_sel @ w_up
        y = g * u @ w_down
        r_sel = _sigmoid(jnp.take_along_axis(r, idx, axis=1))
        y = y * r_sel.reshape(B, C, 1)
        b_off = (jnp.arange(B) * S).reshape(B, 1)
        flat_idx = (idx + b_off).reshape(B * C)
        zero = (x * 0.0).reshape(B * S, D)
        upd = _scatter_add(zero, flat_idx, y.reshape(B * C, D), axis=0)
        return x + upd.reshape(B, S, D)
    x = A_x
    mod = (_silu(c) @ w_mod).reshape(c.shape[0], 6, 1, -1)
    sa, ca, ga, sb, cb, gb = (mod[:, 0].copy(), mod[:, 1].copy(), mod[:, 2].copy(), mod[:, 3].copy(), mod[:, 4].copy(), mod[:, 5].copy())
    h = _layernorm(x, axis=-1) * (1 + ca) + sa
    x = x + ga * _A_ref(h, A_k_cache, A_v_cache, A_wq, A_wo)
    h = _layernorm(x, axis=-1) * (1 + cb) + sb
    x = x + gb * _B_ref(h, B_w_r, B_w_gate, B_w_up, B_w_down)
    return x
```

```python
import functools
import math

import jax
import jax.numpy as jnp
from jax import lax
import jax.experimental.pallas as pl
import jax.experimental.pallas.tpu as pltpu

F32 = jnp.float32
BF16 = jnp.bfloat16

SQ, D = 2048, 1024
HQ, HKV, SK, DH = 32, 4, 2048, 128
W = min(4096, max(256, SK // 4))
REP = HQ // HKV
FF = 3584
EPS = 1e-5
LOG2E = math.log2(math.e)
QSCALE = DH ** -0.5 * LOG2E
GW = REP * DH


def _layernorm(x):
    m = jnp.mean(x, axis=-1, keepdims=True)
    d = x - m
    v = jnp.mean(d * d, axis=-1, keepdims=True)
    return d * lax.rsqrt(v + EPS)


def _make_kernel(BQ):
    NB = SQ // BQ

    def kernel(x_hbm, k_hbm, v_hbm, wq_hbm, wo_hbm, wr_hbm, wg_hbm, wu_hbm, wd_hbm, c_hbm, wm_hbm,
               out_hbm,
               x_v, k_v, kt_v, v_v, wq_v, wo_v, wr_v, wg_v, wu_v, wd_v, c_v, wm_v,
               mod_v, h_v, q_v, o_v, acc_v, x1_v, h2_v, out_v, patch_v, best_v, bidx_v,
               sems, out_sems):
        S_C, S_WR, S_K, S_V, S_WG, S_WU, S_WD, S_PATCH = range(8)
        S_WM = 8
        S_X = 14
        S_WQ = S_X + NB
        S_WO = S_WQ + 4

        def cp_c():
            return pltpu.make_async_copy(c_hbm, c_v, sems.at[S_C])

        def cp_wr():
            return pltpu.make_async_copy(wr_hbm, wr_v, sems.at[S_WR])

        def cp_k():
            return pltpu.make_async_copy(k_hbm.at[:, pl.ds(SK - W, W), :], k_v, sems.at[S_K])

        def cp_v():
            return pltpu.make_async_copy(v_hbm.at[:, pl.ds(SK - W, W), :], v_v, sems.at[S_V])

        def cp_wm(j):
            return pltpu.make_async_copy(wm_hbm.at[:, pl.ds(j * D, D)], wm_v.at[j], sems.at[S_WM + j])

        def cp_x(i):
            return pltpu.make_async_copy(x_hbm.at[pl.ds(i * BQ, BQ), :], x_v.at[pl.ds(i * BQ, BQ), :],
                                         sems.at[S_X + i])

        def cp_wq(g):
            return pltpu.make_async_copy(wq_hbm.at[:, pl.ds(g * GW, GW)], wq_v.at[g], sems.at[S_WQ + g])

        def cp_wo(g):
            return pltpu.make_async_copy(wo_hbm.at[pl.ds(g * GW, GW), :], wo_v.at[g], sems.at[S_WO + g])

        def cp_wg():
            return pltpu.make_async_copy(wg_hbm, wg_v, sems.at[S_WG])

        def cp_wu():
            return pltpu.make_async_copy(wu_hbm, wu_v, sems.at[S_WU])

        def cp_wd():
            return pltpu.make_async_copy(wd_hbm, wd_v, sems.at[S_WD])

        def cp_out(i):
            return pltpu.make_async_copy(out_v.at[pl.ds(i * BQ, BQ), :], out_hbm.at[pl.ds(i * BQ, BQ), :],
                                         out_sems.at[i])

        cp_c().start()
        cp_wm(0).start()
        cp_wm(1).start()
        cp_x(0).start()
        cp_wq(0).start()
        cp_k().start()
        cp_v().start()
        cp_wo(0).start()
        for j in range(2, 6):
            cp_wm(j).start()
        cp_wr().start()
        for g in range(1, 4):
            cp_wq(g).start()
            cp_wo(g).start()
        for i in range(1, NB):
            cp_x(i).start()
        cp_wg().start()
        cp_wu().start()
        cp_wd().start()

        cp_c().wait()
        cf = c_v[...].astype(F32)
        sc = (cf * jax.nn.sigmoid(cf)).astype(BF16)
        sc = jnp.broadcast_to(sc, (16, D))

        def mod_chunk(j):
            cp_wm(j).wait()
            mod_v[j] = jnp.dot(sc, wm_v[j], preferred_element_type=F32)[0:8, :]

        mod_chunk(0)
        mod_chunk(1)

        cp_k().wait()
        for g in range(HKV):
            kt_v[g] = k_v[g].astype(F32).T.astype(BF16)
        cp_v().wait()

        best_v[...] = jnp.full((8, 128), -jnp.inf, F32)
        bidx_v[...] = jnp.zeros((8, 128), jnp.int32)

        def block(i, first):
            rows = pl.ds(pl.multiple_of(i * BQ, BQ), BQ)
            cp_x(i).wait()
            sa = mod_v[0][0:1, :]
            ca = mod_v[1][0:1, :]
            xf = x_v[rows, :].astype(F32)
            h_v[...] = (_layernorm(xf) * (1.0 + ca) + sa).astype(BF16)

            def group(g, first):
                if first:
                    cp_wq(g).wait()
                q = jnp.dot(h_v[...], wq_v[g], preferred_element_type=F32)
                q_v[...] = (q * QSCALE).astype(BF16)
                for hh in range(REP):
                    qh = q_v[:, hh * DH:(hh + 1) * DH]
                    s = jnp.dot(qh, kt_v[g], preferred_element_type=F32)
                    m = jnp.max(s, axis=-1, keepdims=True)
                    p = jnp.exp2(s - m)
                    l = jnp.sum(p, axis=-1, keepdims=True)
                    o = jnp.dot(p.astype(BF16), v_v[g], preferred_element_type=F32)
                    o_v[:, hh * DH:(hh + 1) * DH] = (o * (1.0 / l)).astype(BF16)
                if first:
                    cp_wo(g).wait()
                return jnp.dot(o_v[...], wo_v[g], preferred_element_type=F32)

            if first:
                acc_v[...] = group(0, True)
                for g in range(1, 4):
                    acc_v[...] += group(g, True)
                for j in range(2, 6):
                    mod_chunk(j)
                cp_wr().wait()
            else:
                acc_v[...] = group(0, False)

                def gbody(g, carry):
                    acc_v[...] += group(g, False)
                    return carry
                lax.fori_loop(1, 4, gbody, 0)

            ga = mod_v[2][0:1, :]
            sb = mod_v[3][0:1, :]
            cb = mod_v[4][0:1, :]
            gb = mod_v[5][0:1, :]
            x1 = x_v[rows, :].astype(F32) + ga * acc_v[...]
            h2 = (_layernorm(x1) * (1.0 + cb) + sb).astype(BF16)
            h2f = h2.astype(F32)
            x1_v[rows, :] = x1
            h2_v[rows, :] = h2
            out_v[rows, :] = (x1 + gb * h2f).astype(BF16)
            cp_out(i).start()
            r = jnp.sum(h2f * wr_v[...].astype(F32), axis=-1, keepdims=True)
            r = r.astype(BF16).astype(F32)
            r3 = jnp.broadcast_to(r, (BQ, 128)).reshape(BQ // 8, 8, 128)
            best = best_v[...]
            bidx = bidx_v[...]
            sub = lax.broadcasted_iota(jnp.int32, (8, 128), 0)
            for t in range(BQ // 8):
                rt = r3[t]
                upd = rt > best
                best = jnp.where(upd, rt, best)
                bidx = jnp.where(upd, i * BQ + t * 8 + sub, bidx)
            best_v[...] = best
            bidx_v[...] = bidx

        block(0, True)

        def body(i, carry):
            block(i, False)
            return carry
        lax.fori_loop(1, NB, body, 0)

        best = best_v[...]
        bidx = bidx_v[...]
        mx = jnp.max(best, axis=0, keepdims=True)
        cand = jnp.where(best == mx, bidx, SQ)
        idx = jnp.min(cand)
        idx = jnp.clip(idx, 0, SQ - 1)
        t0 = pl.multiple_of((idx // 16) * 16, 16)
        trow = pl.ds(t0, 16)
        h2t = h2_v[trow, :]
        h2tf = h2t.astype(F32)
        rowid = lax.broadcasted_iota(jnp.int32, (16, D), 0)
        xsel = jnp.where(rowid == idx - t0, h2tf, 0.0).astype(BF16)
        cp_wg().wait()
        gate = jnp.dot(xsel, wg_v[...], preferred_element_type=F32)
        cp_wu().wait()
        up = jnp.dot(xsel, wu_v[...], preferred_element_type=F32)
        act = (gate * jax.nn.sigmoid(gate) * up).astype(BF16)
        cp_wd().wait()
        y = jnp.dot(act, wd_v[...], preferred_element_type=F32)
        rt = jnp.sum(h2tf * wr_v[...].astype(F32), axis=-1, keepdims=True)
        gb = mod_v[5][0:1, :]
        patch_v[...] = (x1_v[trow, :] + gb * (h2tf + y * jax.nn.sigmoid(rt))).astype(BF16)
        for i in range(NB):
            cp_out(i).wait()
        cp = pltpu.make_async_copy(patch_v, out_hbm.at[trow, :], sems.at[S_PATCH])
        cp.start()
        cp.wait()

    return kernel


def _run(A_x, A_k_cache, A_v_cache, A_wq, A_wo, B_x, B_w_r, B_w_gate, B_w_up, B_w_down, c, w_mod,
        BQ=512, flags=None):
    NB = SQ // BQ
    nsem = 14 + NB + 8
    any_spec = pl.BlockSpec(memory_space=pl.ANY)
    out = pl.pallas_call(
        _make_kernel(BQ),
        out_shape=jax.ShapeDtypeStruct((SQ, D), BF16),
        in_specs=[any_spec] * 11,
        out_specs=any_spec,
        scratch_shapes=[
            pltpu.VMEM((SQ, D), BF16),
            pltpu.VMEM((HKV, W, DH), BF16),
            pltpu.VMEM((HKV, DH, W), BF16),
            pltpu.VMEM((HKV, W, DH), BF16),
            pltpu.VMEM((4, D, GW), BF16),
            pltpu.VMEM((4, GW, D), BF16),
            pltpu.VMEM((1, D), BF16),
            pltpu.VMEM((D, FF), BF16),
            pltpu.VMEM((D, FF), BF16),
            pltpu.VMEM((FF, D), BF16),
            pltpu.VMEM((1, D), BF16),
            pltpu.VMEM((6, D, D), BF16),
            pltpu.VMEM((6, 8, D), F32),
            pltpu.VMEM((BQ, D), BF16),
            pltpu.VMEM((BQ, GW), BF16),
            pltpu.VMEM((BQ, GW), BF16),
            pltpu.VMEM((BQ, D), F32),
            pltpu.VMEM((SQ, D), F32),
            pltpu.VMEM((SQ, D), BF16),
            pltpu.VMEM((SQ, D), BF16),
            pltpu.VMEM((16, D), BF16),
            pltpu.VMEM((8, 128), F32),
            pltpu.VMEM((8, 128), jnp.int32),
            pltpu.SemaphoreType.DMA((nsem,)),
            pltpu.SemaphoreType.DMA((NB,)),
        ],
        compiler_params=pltpu.CompilerParams(vmem_limit_bytes=100 * 1024 * 1024, flags=flags),
    )(
        A_x.reshape(SQ, D), A_k_cache.reshape(HKV, SK, DH), A_v_cache.reshape(HKV, SK, DH),
        A_wq, A_wo, B_w_r.reshape(1, D), B_w_gate, B_w_up, B_w_down, c, w_mod,
    )
    return out.reshape(1, SQ, D)


@jax.jit
def pallas_adaLN_cond__sliding_block_cached__moe_arch_mod__prompt_kernel(
    A_x, A_k_cache, A_v_cache, A_wq, A_wo, B_x, B_w_r, B_w_gate, B_w_up, B_w_down, c, w_mod,
):
    return _run(A_x, A_k_cache, A_v_cache, A_wq, A_wo, B_x, B_w_r, B_w_gate, B_w_up, B_w_down, c, w_mod)
```

```python
import contextlib
import math

import jax
import jax.numpy as jnp
from jax import lax
import jax.experimental.pallas as pl
import jax.experimental.pallas.tpu as pltpu

F32 = jnp.float32
BF16 = jnp.bfloat16

SQ, D = 2048, 1024
HQ, HKV, SK, DH = 32, 4, 2048, 128
W = min(4096, max(256, SK // 4))
REP = HQ // HKV
FF = 3584
EPS = 1e-5
LOG2E = math.log2(math.e)
QSCALE = DH ** -0.5 * LOG2E
GW = REP * DH
NG = HKV
LT = 128
DT = D // LT
FT = FF // LT
BQ = 512
NB = SQ // BQ
CH = BQ // NG
PIECE = 16
NST = 2
SW = D // NST


def _layernorm(x):
    m = jnp.mean(x, axis=-1, keepdims=True)
    d = x - m
    v = jnp.mean(d * d, axis=-1, keepdims=True)
    return d * lax.rsqrt(v + EPS)


def _recip(l):
    r = pl.reciprocal(l, approx=True)
    return r * (2.0 - l * r)


def _cat(parts, axis):
    return parts[0] if len(parts) == 1 else jnp.concatenate(parts, axis=axis)


def _make_kernel(NCQ, NCO, PROF, LASTSPLIT, QP, OP, TAILV):
    def scope(name):
        return jax.named_scope(name) if PROF else contextlib.nullcontext()

    def kernel(x_hbm, k_hbm, v_hbm, wq_hbm, wo_hbm, wr_hbm, wg_hbm, wu_hbm, wd_hbm, c_hbm, wm_hbm,
               out_hbm,
               x_v, k_v, v_v, wq_v, wo_v, wr_v, wg_v, wu_v, wd_v, c_v, wm_v, w01_v,
               mod_v, scol_v, n_v, h_a, h_b, q_v, o_v, acc_a, acc_b, x1_v, h2_v, out_v, patch_v, best_v, bidx_v,
               sems, out_sem):
        h_bufs = (h_a, h_b)
        acc_bufs = (acc_a, acc_b)
        S_C, S_WR, S_WG, S_WU, S_WD, S_PATCH, S_X0, S_XR = range(8)
        S_T = 8
        S_X1 = S_T + NST
        S_KV = S_X1 + NG
        S_WO = S_KV + NG
        S_WM = S_WO + NG
        S_WQ = S_WM + NG

        def start(cps):
            for cp in cps if isinstance(cps, list) else [cps]:
                cp.start()

        def wait(cps):
            for cp in cps if isinstance(cps, list) else [cps]:
                cp.wait()

        def coltile(src, r0, nr, t, dst, sem):
            return pltpu.make_async_copy(src.at[pl.ds(r0, nr), pl.ds(pl.multiple_of(t * LT, LT), LT)], dst, sem)

        hpq = REP // NCQ
        cp_c = lambda: pltpu.make_async_copy(c_hbm, c_v, sems.at[S_C])
        cp_wr = lambda: pltpu.make_async_copy(wr_hbm, wr_v, sems.at[S_WR])
        cp_x0 = lambda: pltpu.make_async_copy(x_hbm.at[pl.ds(0, BQ), :], x_v.at[pl.ds(0, BQ), :], sems.at[S_X0])
        cp_xr = lambda: pltpu.make_async_copy(x_hbm.at[pl.ds(2 * BQ, SQ - 2 * BQ), :],
                                              x_v.at[pl.ds(2 * BQ, SQ - 2 * BQ), :], sems.at[S_XR])

        def cp_x1(g):
            rows = pl.ds(pl.multiple_of(BQ + g * CH, CH), CH)
            return pltpu.make_async_copy(x_hbm.at[rows, :], x_v.at[rows, :], sems.at[S_X1 + g])

        def cp_ss(t):
            return [pltpu.make_async_copy(wm_hbm.at[:, pl.ds(pl.multiple_of(j * D + t * SW, SW), SW)],
                                          w01_v.at[j * NST + t], sems.at[S_T + t]) for j in range(2)]

        def cp_kv(g):
            return [pltpu.make_async_copy(k_hbm.at[g, pl.ds(SK - W, W), :], k_v.at[g], sems.at[S_KV + g]),
                    pltpu.make_async_copy(v_hbm.at[g, pl.ds(SK - W, W), :], v_v.at[g], sems.at[S_KV + g])]

        def cp_wq(g, j):
            return [coltile(wq_hbm, 0, D, g * REP + j * hpq + t, wq_v.at[g * REP + j * hpq + t],
                            sems.at[S_WQ + g * NCQ + j]) for t in range(hpq)]

        def cp_wo(g):
            r0 = pl.multiple_of(g * GW, GW)
            return [coltile(wo_hbm, r0, GW, t, wo_v.at[t, pl.ds(r0, GW), :], sems.at[S_WO + g]) for t in range(DT)]

        def cp_wm(g):
            return [coltile(wm_hbm, 0, D, (2 + g) * DT + t, wm_v.at[g * DT + t], sems.at[S_WM + g])
                    for t in range(DT)]

        cp_wg = lambda: [coltile(wg_hbm, 0, D, t, wg_v.at[t], sems.at[S_WG]) for t in range(FT)]
        cp_wu = lambda: [coltile(wu_hbm, 0, D, t, wu_v.at[t], sems.at[S_WU]) for t in range(FT)]
        cp_wd = lambda: [coltile(wd_hbm, 0, FF, t, wd_v.at[t], sems.at[S_WD]) for t in range(DT)]

        def cp_out(r0, n):
            return pltpu.make_async_copy(out_v.at[pl.ds(r0, n), :], out_hbm.at[pl.ds(r0, n), :], out_sem)

        def modrow(j):
            return _cat([mod_v[j, t, 0:1, :] for t in range(DT)], 1)

        def ln1(r0, n, slot, o0):
            xf = x_v[pl.ds(r0, n), :].astype(F32)
            h = (_layernorm(xf) * (1.0 + modrow(1)) + modrow(0)).astype(BF16)
            for t in range(DT):
                h_bufs[slot][t, pl.ds(o0, n), :] = h[:, t * LT:(t + 1) * LT]
            return h

        def epi(r0, n, acc):
            rows = pl.ds(r0, n)
            x1 = x_v[rows, :].astype(F32) + modrow(2) * acc
            h2 = (_layernorm(x1) * (1.0 + modrow(4)) + modrow(3)).astype(BF16)
            h2f = h2.astype(F32)
            x1_v[rows, :] = x1
            h2_v[rows, :] = h2
            out = (x1 + modrow(5) * h2f).astype(BF16)
            out_v[rows, :] = out
            r = jnp.sum(h2f * wr_v[...].astype(F32), axis=-1, keepdims=True)
            r = r.astype(BF16).astype(F32)
            r3 = jnp.broadcast_to(r, (n, 128)).reshape(n // 8, 8, 128)
            sub = lax.broadcasted_iota(jnp.int32, (8, 128), 0) + r0
            best = r3[0]
            bidx = sub
            for t in range(1, n // 8):
                rt = r3[t]
                upd = rt > best
                best = jnp.where(upd, rt, best)
                bidx = jnp.where(upd, sub + t * 8, bidx)
            pslot = r0 // PIECE
            best_v[pslot] = best
            bidx_v[pslot] = bidx
            return out

        def silu_c():
            cf = c_v[...].astype(F32)
            return (cf * jax.nn.sigmoid(cf)).astype(BF16)

        def mod_tiles(j, ts):
            res = []
            for t in ts:
                y = jnp.sum(wm_v[(j - 2) * DT + t].astype(F32) * scol_v[...], axis=0, keepdims=True)
                mod_v[j, t] = jnp.broadcast_to(y, (8, LT))
                res.append(jnp.broadcast_to(y.astype(BF16), (16, LT)))
            return _cat(res, 1)

        def tie_tiles(lhs_tiles, never, dep):
            if dep is None:
                return lhs_tiles
            rows = lhs_tiles[0].shape[0]
            ng = dep.shape[0] // 16
            step = rows // (ng * 16) * 16
            out = []
            for t, lt in enumerate(lhs_tiles):
                if (t + 1) * LT > dep.shape[1]:
                    out.append(lt)
                    continue
                parts = []
                for r in range(ng):
                    a = r * step
                    parts.append(jnp.where(never, dep[r * 16:(r + 1) * 16, t * LT:(t + 1) * LT], lt[a:a + 16]))
                    if step > 16:
                        parts.append(lt[a + 16:a + step])
                if ng * step < rows:
                    parts.append(lt[ng * step:])
                out.append(_cat(parts, 0))
            return out

        def qa_phase(slot, g, never, qdeps, pre_q=None, pre_attn=None):
            hb = h_bufs[slot]
            for j in range(NCQ):
                if pre_q is not None:
                    pre_q(j)
                dep = qdeps[j]() if qdeps and qdeps[j] else None
                lhs = _cat(tie_tiles([hb[t] for t in range(DT)], never, dep), 1)
                w = _cat([wq_v[g * REP + hh] for hh in range(j * hpq, (j + 1) * hpq)], 1)
                q = (jnp.dot(lhs, w, preferred_element_type=F32) * QSCALE).astype(BF16)
                for i_, hh in enumerate(range(j * hpq, (j + 1) * hpq)):
                    q_v[hh] = q[:, i_ * DH:(i_ + 1) * DH]
            if pre_attn is not None:
                pre_attn()
            for hh in range(REP):
                s = lax.dot_general(q_v[hh], k_v[g], (((1,), (1,)), ((), ())), preferred_element_type=F32)
                m = jnp.max(s, axis=-1, keepdims=True)
                p = jnp.exp2(s - m)
                l = jnp.sum(p, axis=-1, keepdims=True)
                o = jnp.dot(p.astype(BF16), v_v[g], preferred_element_type=F32)
                o_v[hh] = (o * _recip(l)).astype(BF16)

        def o_phase(slot, g, never, odeps):
            acc = acc_bufs[slot]
            g0 = pl.multiple_of(g * GW, GW)
            npc = DT // NCO
            for j in range(NCO):
                dep = odeps[j]() if odeps and odeps[j] else None
                lhs = _cat(tie_tiles([o_v[t] for t in range(REP)], never, dep), 1)
                w = _cat([wo_v[n, pl.ds(g0, GW), :] for n in range(j * npc, (j + 1) * npc)], 1)
                d = jnp.dot(lhs, w, preferred_element_type=F32)
                cs = slice(j * npc * LT, (j + 1) * npc * LT)
                acc[:, cs] = jnp.where(g == 0, 0.0, acc[:, cs]) + d

        with scope("pro"):
            start(cp_c())
            start(cp_x0())
            for t in range(NST):
                start(cp_ss(t))
            for j in range(NCQ):
                start(cp_wq(0, j))
                if j == 0:
                    start(cp_x1(0))
                if j == 1:
                    start(cp_kv(0))

            best_v[...] = jnp.full(best_v.shape, -jnp.inf, F32)
            bidx_v[...] = jnp.zeros(bidx_v.shape, jnp.int32)

            wait(cp_c())
            wait(cp_x0())

            def ln_body(r, carry):
                r0 = pl.multiple_of(r * CH, CH)
                n = _layernorm(x_v[pl.ds(r0, CH), :].astype(F32))
                for t in range(DT):
                    n_v[t, pl.ds(r0, CH), :] = n[:, t * LT:(t + 1) * LT]
                return carry
            lax.fori_loop(0, BQ // CH, ln_body, 0)
            start(cp_wo(0))
            start(cp_wm(0))
            start(cp_wr())
            scol_v[...] = jnp.broadcast_to(silu_c().astype(F32), (LT, D)).T

            def tile_body(t, carry):
                wait(cp_ss(t))
                sc = jnp.broadcast_to(silu_c(), (16, D))
                sa = jnp.dot(sc, w01_v[t], preferred_element_type=F32)[0:8, :]
                ca = jnp.dot(sc, w01_v[NST + t], preferred_element_type=F32)[0:8, :]
                for u in range(SW // LT):
                    tt = t * (SW // LT) + u
                    cs = slice(u * LT, (u + 1) * LT)
                    mod_v[0, tt] = sa[:, cs]
                    mod_v[1, tt] = ca[:, cs]
                    h_a[tt] = (n_v[tt] * (1.0 + ca[0:1, cs]) + sa[0:1, cs]).astype(BF16)
                return carry
            lax.fori_loop(0, NST, tile_body, 0)

        def pieces(n, k):
            t = n // 16
            sizes = [(t // k + (1 if a < t % k else 0)) * 16 for a in range(k)]
            offs = [sum(sizes[:a]) for a in range(k)]
            return list(zip(offs, sizes))

        for i in range(NB):
            slot = i % 2

            def body(g, carry, i=i, slot=slot, fine=False):
                never = g < 0

                def ln_piece(o, n):
                    o0 = pl.multiple_of(g * CH + o, 16)
                    return ln1(pl.multiple_of((i + 1) * BQ + o0, 16), n, 1 - slot, o0)

                def epi_piece(o, n):
                    o0 = pl.multiple_of(g * CH + o, 16)
                    return epi(pl.multiple_of((i - 1) * BQ + o0, 16), n, acc_bufs[1 - slot][pl.ds(o0, n), :])

                def both(o, n):
                    def f():
                        e = None
                        if i > 0:
                            e = epi_piece(o, n)
                        if i + 1 < NB:
                            hv = ln_piece(o, n)
                            e = hv if e is None else jnp.where(never, hv, e)
                        return e
                    return f

                qd = [None] * NCQ
                od = [None] * NCO
                qpts = list(range(NCQ - QP, NCQ))
                opts = list(range(OP))
                allp = pieces(CH, QP + OP)
                for k, j in enumerate(qpts):
                    qd[j] = both(*allp[k])
                if i > 0 or OP:
                    for k, j in enumerate(opts):
                        od[j] = both(*allp[QP + k])

                pre_q = pre_attn = None
                if i == 0:
                    @pl.when(g + 1 < NG)
                    def _():
                        for j in range(NCQ):
                            start(cp_wq(g + 1, j))
                        start(cp_kv(g + 1))
                        start(cp_x1(g + 1))
                        start(cp_wo(g + 1))
                        start(cp_wm(g + 1))

                    @pl.when(g == NG - 2)
                    def _():
                        start(cp_xr())
                    if fine:
                        def pre_q(j):
                            with scope(f"w_wq{j}"):
                                wait(cp_wq(g, j))
                                if j == 1:
                                    wait(cp_x1(g))

                        def pre_attn():
                            with scope("w_kv"):
                                wait(cp_kv(g))
                    else:
                        wait(cp_x1(g))
                        for j in range(NCQ):
                            wait(cp_wq(g, j))
                        wait(cp_kv(g))
                        wait(cp_wo(g))
                        wait(cp_wm(g))
                    tpo = DT // NCO

                    def with_mod(j, prev):
                        def f():
                            ts = list(range(j * tpo, (j + 1) * tpo))
                            y = mod_tiles(2 + g, ts)
                            if prev is None:
                                return y
                            e = prev()
                            top = jnp.where(never, y, e[0:16, 0:y.shape[1]])
                            return _cat([_cat([top, e[0:16, y.shape[1]:]], 1), e[16:]], 0)
                        return f
                    od = [with_mod(j, od[j]) for j in range(NCO)]

                qa_phase(slot, g, never, qd, pre_q, pre_attn)
                if i == 0 and fine:
                    with scope("w_wo"):
                        wait(cp_wo(g))
                        wait(cp_wm(g))
                o_phase(slot, g, never, od)
                if i > 0:
                    cp_out(pl.multiple_of((i - 1) * BQ + g * CH, CH), CH).start()
                return carry

            if i == 0:
                with scope("unit0"):
                    body(pl.program_id(0), 0, fine=True)
                with scope("blk0"):
                    lax.fori_loop(1, NG, body, 0)
            else:
                with scope(f"blk{i}"):
                    lax.fori_loop(0, NG, body, 0)
            if i == 0:
                with scope("mid"):
                    wait(cp_wr())
                    wait(cp_xr())
                    start(cp_wg())
                    start(cp_wu())
                    start(cp_wd())

        last = NB - 1
        with scope("lastepi"):
            for o in range(0, BQ, CH):
                epi(last * BQ + o, CH, acc_bufs[last % 2][o:o + CH, :])
            cp_out(last * BQ, BQ).start()

        with scope("tail"):
            ent = [(best_v[t], bidx_v[t]) for t in range(SQ // PIECE)]
            while len(ent) > 1:
                nxt = []
                for t in range(0, len(ent), 2):
                    (b0_, i0_), (b1_, i1_) = ent[t], ent[t + 1]
                    upd = b1_ > b0_
                    nxt.append((jnp.where(upd, b1_, b0_), jnp.where(upd, i1_, i0_)))
                ent = nxt
            best, bidx = ent[0]
            mx = jnp.max(best, axis=0, keepdims=True)
            cand = jnp.where(best == mx, bidx, SQ)
            idx = jnp.clip(jnp.min(cand), 0, SQ - 1)
            t0 = pl.multiple_of((idx // 16) * 16, 16)
            trow = pl.ds(t0, 16)
            h2tf = h2_v[trow, :].astype(F32)
            rowid = lax.broadcasted_iota(jnp.int32, (16, D), 0)
            xsel = jnp.where(rowid == idx - t0, h2tf, 0.0).astype(BF16)
            with scope("t_gu"):
                wait(cp_wg())
                gate = jnp.dot(xsel, _cat([wg_v[t] for t in range(FT)], 1), preferred_element_type=F32)
                wait(cp_wu())
                up = jnp.dot(xsel, _cat([wu_v[t] for t in range(FT)], 1), preferred_element_type=F32)
                act = (gate * jax.nn.sigmoid(gate) * up).astype(BF16)
            with scope("t_d"):
                wait(cp_wd())
                y = jnp.dot(act, _cat([wd_v[t] for t in range(DT)], 1), preferred_element_type=F32)
            with scope("t_p"):
                rt = jnp.sum(h2tf * wr_v[...].astype(F32), axis=-1, keepdims=True)
                patch_v[...] = (x1_v[trow, :] + modrow(5) * (h2tf + y * jax.nn.sigmoid(rt))).astype(BF16)
                cp_out(0, SQ).wait()
                cp = pltpu.make_async_copy(patch_v, out_hbm.at[trow, :], sems.at[S_PATCH])
                cp.start()
                cp.wait()

    return kernel


def _run(A_x, A_k_cache, A_v_cache, A_wq, A_wo, B_x, B_w_r, B_w_gate, B_w_up, B_w_down, c, w_mod,
        NCQ=4, NCO=4, PROF=False, LASTSPLIT=False, QP=3, OP=0, TAILV=0, flags=None):
    nsem = 8 + NST + 4 * NG + NG * NCQ
    any_spec = pl.BlockSpec(memory_space=pl.ANY)
    out = pl.pallas_call(
        _make_kernel(NCQ, NCO, PROF, LASTSPLIT, QP, OP, TAILV),
        out_shape=jax.ShapeDtypeStruct((SQ, D), BF16),
        grid=(1,),
        in_specs=[any_spec] * 11,
        out_specs=any_spec,
        scratch_shapes=[
            pltpu.VMEM((SQ, D), BF16),
            pltpu.VMEM((HKV, W, DH), BF16),
            pltpu.VMEM((HKV, W, DH), BF16),
            pltpu.VMEM((HQ, D, LT), BF16),
            pltpu.VMEM((DT, HQ * DH, LT), BF16),
            pltpu.VMEM((1, D), BF16),
            pltpu.VMEM((FT, D, LT), BF16),
            pltpu.VMEM((FT, D, LT), BF16),
            pltpu.VMEM((DT, FF, LT), BF16),
            pltpu.VMEM((1, D), BF16),
            pltpu.VMEM((4 * DT, D, LT), BF16),
            pltpu.VMEM((2 * NST, D, SW), BF16),
            pltpu.VMEM((6, DT, 8, LT), F32),
            pltpu.VMEM((D, LT), F32),
            pltpu.VMEM((DT, BQ, LT), F32),
            pltpu.VMEM((DT, BQ, LT), BF16),
            pltpu.VMEM((DT, BQ, LT), BF16),
            pltpu.VMEM((REP, BQ, LT), BF16),
            pltpu.VMEM((REP, BQ, LT), BF16),
            pltpu.VMEM((BQ, D), F32),
            pltpu.VMEM((BQ, D), F32),
            pltpu.VMEM((SQ, D), F32),
            pltpu.VMEM((SQ, D), BF16),
            pltpu.VMEM((SQ, D), BF16),
            pltpu.VMEM((16, D), BF16),
            pltpu.VMEM((SQ // PIECE, 8, 128), F32),
            pltpu.VMEM((SQ // PIECE, 8, 128), jnp.int32),
            pltpu.SemaphoreType.DMA((nsem,)),
            pltpu.SemaphoreType.DMA(()),
        ],
        compiler_params=pltpu.CompilerParams(vmem_limit_bytes=110 * 1024 * 1024, flags=flags),
    )(
        A_x.reshape(SQ, D), A_k_cache.reshape(HKV, SK, DH), A_v_cache.reshape(HKV, SK, DH),
        A_wq, A_wo, B_w_r.reshape(1, D), B_w_gate, B_w_up, B_w_down, c, w_mod,
    )
    return out.reshape(1, SQ, D)


@jax.jit
def pallas_adaLN_cond__sliding_block_cached__moe_arch_mod__prompt_kernel(
    A_x, A_k_cache, A_v_cache, A_wq, A_wo, B_x, B_w_r, B_w_gate, B_w_up, B_w_down, c, w_mod,
):
    return _run(A_x, A_k_cache, A_v_cache, A_wq, A_wo, B_x, B_w_r, B_w_gate, B_w_up, B_w_down, c, w_mod)
```

```python
import contextlib
import math

import jax
import jax.numpy as jnp
from jax import lax
import jax.experimental.pallas as pl
import jax.experimental.pallas.tpu as pltpu

F32 = jnp.float32
BF16 = jnp.bfloat16

SQ, D = 2048, 1024
HQ, HKV, SK, DH = 32, 4, 2048, 128
W = min(4096, max(256, SK // 4))
REP = HQ // HKV
FF = 3584
EPS = 1e-5
LOG2E = math.log2(math.e)
QSCALE = DH ** -0.5 * LOG2E
GW = REP * DH
NG = HKV
LT = 128
DT = D // LT
FT = FF // LT
BQ = 512
NB = SQ // BQ
CH = BQ // NG
PIECE = 16
NST = 2
SW = D // NST


def _layernorm(x):
    m = jnp.mean(x, axis=-1, keepdims=True)
    d = x - m
    v = jnp.mean(d * d, axis=-1, keepdims=True)
    return d * lax.rsqrt(v + EPS)


def _recip(l):
    r = pl.reciprocal(l, approx=True)
    return r * (2.0 - l * r)


def _cat(parts, axis):
    return parts[0] if len(parts) == 1 else jnp.concatenate(parts, axis=axis)


def _make_kernel(NCQ, NCO, PROF, LASTSPLIT, QP, OP, TAILV, LAG, LSUM, MODPOS, MT, MR, MSPLIT):
    def scope(name):
        return jax.named_scope(name) if PROF else contextlib.nullcontext()

    def kernel(x_hbm, k_hbm, v_hbm, wq_hbm, wo_hbm, wr_hbm, wg_hbm, wu_hbm, wd_hbm, c_hbm, wm_hbm,
               out_hbm,
               x_v, k_v, v_v, wq_v, wo_v, wr_v, wg_v, wu_v, wd_v, c_v, wm_v, w01_v,
               mod_v, scol_v, col_v, n_v, h_a, h_b, q_v, o_v, acc_a, acc_b, x1_v, h2_v, out_v, patch_v, best_v, bidx_v,
               sems, out_sem):
        h_bufs = (h_a, h_b)
        acc_bufs = (acc_a, acc_b)
        S_C, S_WR, S_WG, S_WU, S_WD, S_PATCH, S_X0, S_XR = range(8)
        S_T = 8
        S_X1 = S_T + NST
        S_KV = S_X1 + NG
        S_WO = S_KV + NG
        S_WM = S_WO + NG
        S_WQ = S_WM + NG

        def start(cps):
            for cp in cps if isinstance(cps, list) else [cps]:
                cp.start()

        def wait(cps):
            for cp in cps if isinstance(cps, list) else [cps]:
                cp.wait()

        def coltile(src, r0, nr, t, dst, sem):
            return pltpu.make_async_copy(src.at[pl.ds(r0, nr), pl.ds(pl.multiple_of(t * LT, LT), LT)], dst, sem)

        hpq = REP // NCQ
        cp_c = lambda: pltpu.make_async_copy(c_hbm, c_v, sems.at[S_C])
        cp_wr = lambda: pltpu.make_async_copy(wr_hbm, wr_v, sems.at[S_WR])
        cp_x0 = lambda: pltpu.make_async_copy(x_hbm.at[pl.ds(0, BQ), :], x_v.at[pl.ds(0, BQ), :], sems.at[S_X0])
        cp_xr = lambda: pltpu.make_async_copy(x_hbm.at[pl.ds(2 * BQ, SQ - 2 * BQ), :],
                                              x_v.at[pl.ds(2 * BQ, SQ - 2 * BQ), :], sems.at[S_XR])

        def cp_x1(g):
            rows = pl.ds(pl.multiple_of(BQ + g * CH, CH), CH)
            return pltpu.make_async_copy(x_hbm.at[rows, :], x_v.at[rows, :], sems.at[S_X1 + g])

        def cp_ss(t):
            return [pltpu.make_async_copy(wm_hbm.at[:, pl.ds(pl.multiple_of(j * D + t * SW, SW), SW)],
                                          w01_v.at[j * NST + t], sems.at[S_T + t]) for j in range(2)]

        def cp_kv(g):
            return [pltpu.make_async_copy(k_hbm.at[g, pl.ds(SK - W, W), :], k_v.at[g], sems.at[S_KV + g]),
                    pltpu.make_async_copy(v_hbm.at[g, pl.ds(SK - W, W), :], v_v.at[g], sems.at[S_KV + g])]

        def cp_wq(g, j):
            return [coltile(wq_hbm, 0, D, g * REP + j * hpq + t, wq_v.at[g * REP + j * hpq + t],
                            sems.at[S_WQ + g * NCQ + j]) for t in range(hpq)]

        def cp_wo(g):
            r0 = pl.multiple_of(g * GW, GW)
            return [coltile(wo_hbm, r0, GW, t, wo_v.at[t, pl.ds(r0, GW), :], sems.at[S_WO + g]) for t in range(DT)]

        def cp_wm(g):
            return [coltile(wm_hbm, 0, D, (2 + g) * DT + t, wm_v.at[g * DT + t], sems.at[S_WM + g])
                    for t in range(DT)]

        cp_wg = lambda: [coltile(wg_hbm, 0, D, t, wg_v.at[t], sems.at[S_WG]) for t in range(FT)]
        cp_wu = lambda: [coltile(wu_hbm, 0, D, t, wu_v.at[t], sems.at[S_WU]) for t in range(FT)]
        cp_wd = lambda: [coltile(wd_hbm, 0, FF, t, wd_v.at[t], sems.at[S_WD]) for t in range(DT)]

        def cp_out(r0, n):
            return pltpu.make_async_copy(out_v.at[pl.ds(r0, n), :], out_hbm.at[pl.ds(r0, n), :], out_sem)

        def modrow(j):
            return _cat([mod_v[j, t, 0:1, :] for t in range(DT)], 1)

        def wr_row():
            w = wr_v[...].astype(F32)
            return _cat([w[t:t + 1, :] for t in range(DT)], 1)

        def ln1(r0, n, slot, o0):
            xf = x_v[pl.ds(r0, n), :].astype(F32)
            h = (_layernorm(xf) * (1.0 + modrow(1)) + modrow(0)).astype(BF16)
            for t in range(DT):
                h_bufs[slot][t, pl.ds(o0, n), :] = h[:, t * LT:(t + 1) * LT]
            return h

        def epi(r0, n, acc):
            rows = pl.ds(r0, n)
            x1 = x_v[rows, :].astype(F32) + modrow(2) * acc
            h2 = (_layernorm(x1) * (1.0 + modrow(4)) + modrow(3)).astype(BF16)
            h2f = h2.astype(F32)
            x1_v[rows, :] = x1
            h2_v[rows, :] = h2
            out = (x1 + modrow(5) * h2f).astype(BF16)
            out_v[rows, :] = out
            r = jnp.sum(h2f * wr_row(), axis=-1, keepdims=True)
            r = r.astype(BF16).astype(F32)
            r3 = jnp.broadcast_to(r, (n, 128)).reshape(n // 8, 8, 128)
            sub = lax.broadcasted_iota(jnp.int32, (8, 128), 0) + r0
            best = r3[0]
            bidx = sub
            for t in range(1, n // 8):
                rt = r3[t]
                upd = rt > best
                best = jnp.where(upd, rt, best)
                bidx = jnp.where(upd, sub + t * 8, bidx)
            pslot = r0 // PIECE
            best_v[pslot] = best
            bidx_v[pslot] = bidx
            return out

        def silu_c():
            cf = c_v[...].astype(F32)
            return (cf * jax.nn.sigmoid(cf)).astype(BF16)

        def mod_tiles(j, ts, parts=None):
            res = []
            for t in ts:
                if parts is None:
                    y = jnp.sum(wm_v[(j - 2) * DT + t].astype(F32) * scol_v[...], axis=0, keepdims=True)
                else:
                    acc8 = None
                    kq = D // MSPLIT
                    for k_ in range(MSPLIT):
                        rs = slice(k_ * kq, (k_ + 1) * kq)
                        pr = wm_v[(j - 2) * DT + t, rs, :].astype(F32) * scol_v[rs, :]
                        p8 = pr.reshape(kq // 8, 8, LT).sum(axis=0)
                        parts.append(jnp.concatenate([p8, p8], axis=0).astype(BF16))
                        acc8 = p8 if acc8 is None else acc8 + p8
                    y = jnp.sum(acc8, axis=0, keepdims=True)
                mod_v[j, t] = jnp.broadcast_to(y, (8, LT))
                res.append(jnp.broadcast_to(y.astype(BF16), (16, LT)))
            return _cat(res, 1)

        def tie_tiles(lhs_tiles, never, dep):
            if dep is None:
                return lhs_tiles
            if isinstance(dep, list):
                out = list(lhs_tiles)
                for (t, a, val) in dep:
                    lt = out[t]
                    out[t] = _cat(([lt[0:a]] if a else []) + [jnp.where(never, val, lt[a:a + 16])] +
                                  ([lt[a + 16:]] if a + 16 < lt.shape[0] else []), 0)
                return out
            rows = lhs_tiles[0].shape[0]
            ng = dep.shape[0] // 16
            step = rows // (ng * 16) * 16
            out = []
            for t, lt in enumerate(lhs_tiles):
                if (t + 1) * LT > dep.shape[1]:
                    out.append(lt)
                    continue
                parts = []
                for r in range(ng):
                    a = r * step
                    parts.append(jnp.where(never, dep[r * 16:(r + 1) * 16, t * LT:(t + 1) * LT], lt[a:a + 16]))
                    if step > 16:
                        parts.append(lt[a + 16:a + step])
                if ng * step < rows:
                    parts.append(lt[ng * step:])
                out.append(_cat(parts, 0))
            return out

        def qa_phase(slot, g, never, qdeps, pre_q=None, pre_attn=None, hdeps=None):
            hb = h_bufs[slot]
            for j in range(NCQ):
                if pre_q is not None:
                    pre_q(j)
                dep = qdeps[j]() if qdeps and qdeps[j] else None
                lhs = _cat(tie_tiles([hb[t] for t in range(DT)], never, dep), 1)
                w = _cat([wq_v[g * REP + hh] for hh in range(j * hpq, (j + 1) * hpq)], 1)
                q = (jnp.dot(lhs, w, preferred_element_type=F32) * QSCALE).astype(BF16)
                for i_, hh in enumerate(range(j * hpq, (j + 1) * hpq)):
                    q_v[hh] = q[:, i_ * DH:(i_ + 1) * DH]
            if pre_attn is not None:
                pre_attn()
            for hh in range(REP):
                qh = q_v[hh]
                if hdeps is not None and hdeps[hh] is not None:
                    qh = tie_tiles([qh], never, hdeps[hh]())[0]
                s = lax.dot_general(qh, k_v[g], (((1,), (1,)), ((), ())), preferred_element_type=F32)
                m = jnp.max(s, axis=-1, keepdims=True)
                p = jnp.exp2(s - m)
                pb = p.astype(BF16)
                if LSUM == 0:
                    l = jnp.sum(p, axis=-1, keepdims=True)
                elif LSUM == 1:
                    ps = p[:, 0:LT] + p[:, LT:2 * LT] + p[:, 2 * LT:3 * LT] + p[:, 3 * LT:4 * LT]
                    l = jnp.sum(ps, axis=-1, keepdims=True)
                    pb = jnp.concatenate([jnp.where(never, ps.astype(BF16), pb[:, 0:LT]), pb[:, LT:]], axis=1)
                elif LSUM == 2:
                    l = jnp.sum(pb.astype(F32), axis=-1, keepdims=True)
                elif LSUM == 3:
                    l = jnp.sum(p, axis=-1, keepdims=True)
                    r_ = _recip(l)
                    pb = jnp.concatenate([jnp.where(never, jnp.broadcast_to(r_, (BQ, LT)).astype(BF16), pb[:, 0:LT]),
                                          pb[:, LT:]], axis=1)
                o = jnp.dot(pb, v_v[g], preferred_element_type=F32)
                o_v[hh] = (o * _recip(l)).astype(BF16)

        def o_phase(slot, g, never, odeps):
            acc = acc_bufs[slot]
            g0 = pl.multiple_of(g * GW, GW)
            npc = DT // NCO
            for j in range(NCO):
                dep = odeps[j]() if odeps and odeps[j] else None
                lhs = _cat(tie_tiles([o_v[t] for t in range(REP)], never, dep), 1)
                w = _cat([wo_v[n, pl.ds(g0, GW), :] for n in range(j * npc, (j + 1) * npc)], 1)
                d = jnp.dot(lhs, w, preferred_element_type=F32)
                cs = slice(j * npc * LT, (j + 1) * npc * LT)
                acc[:, cs] = jnp.where(g == 0, 0.0, acc[:, cs]) + d

        def o_phase_final(slot, g, never):
            acc = acc_bufs[slot]
            g0 = pl.multiple_of(g * GW, GW)
            sizes = [BQ // LASTSPLIT] * LASTSPLIT if isinstance(LASTSPLIT, int) else list(LASTSPLIT)
            assert sum(sizes) == BQ
            dep = None
            r0 = 0
            for rc in sizes:
                rows = slice(r0, r0 + rc)
                lts = [o_v[t, rows, :] for t in range(REP)]
                if dep is not None and dep.shape[0] > rc:
                    parts = [dep[a:a + rc] for a in range(0, dep.shape[0] - rc + 1, rc)]
                    if dep.shape[0] % rc:
                        parts.append(dep[dep.shape[0] - rc:])
                    dep = parts[0]
                    for p_ in parts[1:]:
                        dep = jnp.where(never, p_, dep)
                lhs = _cat(tie_tiles(lts, never, dep), 1)
                w = _cat([wo_v[n, pl.ds(g0, GW), :] for n in range(DT)], 1)
                d = acc[rows, :] + jnp.dot(lhs, w, preferred_element_type=F32)
                dep = epi((NB - 1) * BQ + r0, rc, d)
                r0 += rc

        with scope("pro"):
            start(cp_c())
            start(cp_x0())
            for t in range(NST):
                start(cp_ss(t))
            for j in range(NCQ):
                start(cp_wq(0, j))
                if j == 0:
                    start(cp_x1(0))
                if j == 1:
                    start(cp_kv(0))

            best_v[...] = jnp.full(best_v.shape, -jnp.inf, F32)
            bidx_v[...] = jnp.zeros(bidx_v.shape, jnp.int32)

            wait(cp_c())
            wait(cp_x0())

            def ln_body(r, carry):
                r0 = pl.multiple_of(r * CH, CH)
                n = _layernorm(x_v[pl.ds(r0, CH), :].astype(F32))
                for t in range(DT):
                    n_v[t, pl.ds(r0, CH), :] = n[:, t * LT:(t + 1) * LT]
                return carry
            lax.fori_loop(0, BQ // CH, ln_body, 0)
            start(cp_wo(0))
            start(cp_wm(0))
            start(cp_wr())
            scol_v[...] = jnp.broadcast_to(silu_c().astype(F32), (LT, D)).T

            def tile_body(t, carry):
                wait(cp_ss(t))
                sc = jnp.broadcast_to(silu_c(), (16, D))
                sa = jnp.dot(sc, w01_v[t], preferred_element_type=F32)[0:8, :]
                ca = jnp.dot(sc, w01_v[NST + t], preferred_element_type=F32)[0:8, :]
                for u in range(SW // LT):
                    tt = t * (SW // LT) + u
                    cs = slice(u * LT, (u + 1) * LT)
                    mod_v[0, tt] = sa[:, cs]
                    mod_v[1, tt] = ca[:, cs]
                    h_a[tt] = (n_v[tt] * (1.0 + ca[0:1, cs]) + sa[0:1, cs]).astype(BF16)
                return carry
            lax.fori_loop(0, NST, tile_body, 0)

        def pieces(n, k):
            t = n // 16
            sizes = [(t // k + (1 if a < t % k else 0)) * 16 for a in range(k)]
            offs = [sum(sizes[:a]) for a in range(k)]
            return list(zip(offs, sizes))

        for i in range(NB):
            slot = i % 2

            def body(g, carry, i=i, slot=slot, fine=False, final=False):
                never = g < 0

                def ln_piece(o, n):
                    o0 = pl.multiple_of(g * CH + o, 16)
                    return ln1(pl.multiple_of((i + 1) * BQ + o0, 16), n, 1 - slot, o0)

                def epi_piece(o, n):
                    o0 = pl.multiple_of(g * CH + o, 16)
                    return epi(pl.multiple_of((i - 1) * BQ + o0, 16), n, acc_bufs[1 - slot][pl.ds(o0, n), :])

                def both(o, n):
                    def f():
                        e = None
                        if i > 0:
                            e = epi_piece(o, n)
                        if i + 1 < NB:
                            hv = ln_piece(o, n)
                            e = hv if e is None else jnp.where(never, hv, e)
                        return e
                    return f

                qd = [None] * NCQ
                od = [None] * NCO
                qpts = list(range(NCQ - QP, NCQ))
                opts = list(range(OP))
                allp = pieces(CH, QP + OP)
                for k, j in enumerate(qpts):
                    qd[j] = both(*allp[k])
                if i > 0 or OP:
                    for k, j in enumerate(opts):
                        od[j] = both(*allp[QP + k])

                pre_q = pre_attn = None
                if i == 0:
                    @pl.when(g + 1 < NG)
                    def _():
                        for j in range(NCQ):
                            start(cp_wq(g + 1, j))
                        start(cp_kv(g + 1))
                        start(cp_x1(g + 1))
                        start(cp_wo(g + 1))
                        start(cp_wm(g + 1))

                    @pl.when(g == NG - 2)
                    def _():
                        start(cp_xr())
                    if fine:
                        def pre_q(j):
                            with scope(f"w_wq{j}"):
                                wait(cp_wq(g, j))
                                if j == 1:
                                    wait(cp_x1(g))

                        def pre_attn():
                            with scope("w_kv"):
                                wait(cp_kv(g))
                    else:
                        wait(cp_x1(g))
                        for j in range(NCQ):
                            wait(cp_wq(g, j))
                        wait(cp_kv(g))
                        wait(cp_wo(g))
                        wait(cp_wm(g))
                    tpo = DT // NCO

                    def with_mod(j, prev):
                        def f():
                            ts = list(range(j * tpo, (j + 1) * tpo))
                            if MSPLIT > 1 and prev is None:
                                parts = []
                                y = mod_tiles(2 + g, ts, parts)
                                deps = []
                                for k_, pv in enumerate(parts[:-1]):
                                    pos = (k_ + 1) * 64 // len(parts)
                                    deps.append(((0 if pos < 32 else 4) + k_ % 4, (pos % 32) * 16, pv))
                                deps.append((7, 496, y[:, 0:LT]))
                                return deps
                            y = mod_tiles(2 + g, ts)
                            if prev is None:
                                return [((MT + k_) % REP, MR, y[:, k_ * LT:(k_ + 1) * LT]) for k_ in range(len(ts))]
                            e = prev()
                            top = jnp.where(never, y, e[0:16, 0:y.shape[1]])
                            return _cat([_cat([top, e[0:16, y.shape[1]:]], 1), e[16:]], 0)
                        return f
                    hd = None
                    if MODPOS == 'o':
                        od = [with_mod(j, od[j]) for j in range(NCO)]
                    elif MODPOS == 'attn':
                        hd = [(lambda t=t: mod_tiles(2 + g, [t])) for t in range(DT)]
                        if fine:
                            pa = pre_attn

                            def pre_attn():
                                pa()
                                wait(cp_wm(g))
                    elif MODPOS == 'mix':
                        hd = [(lambda t=t: mod_tiles(2 + g, [t // 2])) if t % 2 == 1 else None for t in range(REP)]
                        od = [(lambda t=t: mod_tiles(2 + g, [DT // 2 + t // 2])) if t % 2 == 0 else None for t in range(NCO)]
                        if fine:
                            pa = pre_attn

                            def pre_attn():
                                pa()
                                wait(cp_wm(g))
                else:
                    hd = None

                qa_phase(slot, g, never, qd, pre_q, pre_attn, hd)
                if i == 0 and fine:
                    with scope("w_wo"):
                        wait(cp_wo(g))
                        if MODPOS == 'o':
                            wait(cp_wm(g))
                if final:
                    o_phase_final(slot, g, never)
                else:
                    o_phase(slot, g, never, od)
                if i > 0:
                    cp_out(pl.multiple_of((i - 1) * BQ + g * CH, CH), CH).start()
                return carry

            if i == 0:
                with scope("unit0"):
                    body(pl.program_id(0), 0, fine=True)
                with scope("blk0"):
                    lax.fori_loop(1, NG, body, 0)
            elif i == NB - 1 and LASTSPLIT:
                with scope(f"blk{i}"):
                    lax.fori_loop(0, NG - 1, body, 0)
                with scope("unitL"):
                    body(pl.program_id(0) + (NG - 1), 0, final=True)
            else:
                with scope(f"blk{i}"):
                    lax.fori_loop(0, NG, body, 0)
            if i == 0:
                with scope("mid"):
                    wait(cp_wr())
                    wait(cp_xr())
                    start(cp_wg())
                    start(cp_wu())
                    start(cp_wd())

        last = NB - 1
        with scope("lastepi"):
            if not LASTSPLIT:
                for o in range(0, BQ, CH):
                    epi(last * BQ + o, CH, acc_bufs[last % 2][o:o + CH, :])
            cp_out(last * BQ, BQ).start()

        with scope("tail"):
            ent = [(best_v[t], bidx_v[t]) for t in range(SQ // PIECE)]
            while len(ent) > 1:
                nxt = []
                for t in range(0, len(ent), 2):
                    (b0_, i0_), (b1_, i1_) = ent[t], ent[t + 1]
                    upd = b1_ > b0_
                    nxt.append((jnp.where(upd, b1_, b0_), jnp.where(upd, i1_, i0_)))
                ent = nxt
            best, bidx = ent[0]
            mx = jnp.max(best, axis=0, keepdims=True)
            cand = jnp.where(best == mx, bidx, SQ)
            idx = jnp.clip(jnp.min(cand), 0, SQ - 1)
            t0 = pl.multiple_of((idx // 16) * 16, 16)
            trow = pl.ds(t0, 16)
            h2tf = h2_v[trow, :].astype(F32)
            rowid = lax.broadcasted_iota(jnp.int32, (16, D), 0)
            xsel = jnp.where(rowid == idx - t0, h2tf, 0.0)
            if TAILV == 0:
                xsel = xsel.astype(BF16)
                with scope("t_gu"):
                    wait(cp_wg())
                    gate = jnp.dot(xsel, _cat([wg_v[t] for t in range(FT)], 1), preferred_element_type=F32)
                    wait(cp_wu())
                    up = jnp.dot(xsel, _cat([wu_v[t] for t in range(FT)], 1), preferred_element_type=F32)
                    act = (gate * jax.nn.sigmoid(gate) * up).astype(BF16)
                with scope("t_d"):
                    wait(cp_wd())
                    y = jnp.dot(act, _cat([wd_v[t] for t in range(DT)], 1), preferred_element_type=F32)
            else:
                never = idx < 0
                nB = TAILV
                nA = FT - nB
                xrow = jnp.sum(xsel, axis=0, keepdims=True)
                x16 = jnp.broadcast_to(xrow, (16, D)).astype(BF16)
                col_v[0:D, :] = jnp.broadcast_to(xrow, (LT, D)).T

                def colsum(p):
                    n = p.shape[0]
                    p = p.reshape(n // 64, 64, LT).sum(axis=0)
                    p = p.reshape(8, 8, LT).sum(axis=0)
                    return jnp.sum(p, axis=0, keepdims=True)

                def vpu_tile(w_ref, t, c0, n):
                    return colsum(w_ref[t, 0:n, :].astype(F32) * col_v[c0:c0 + n, :])

                def tie_w(w, res):
                    top = jnp.where(never, jnp.broadcast_to(res.astype(BF16), (16, LT)), w[0:16])
                    return jnp.concatenate([top, w[16:]], axis=0)

                with scope("t_gu"):
                    wait(cp_wg())
                    wait(cp_wu())
                    vjobs = [(wg_v, nA + b) for b in range(nB)] + [(wu_v, nA + b) for b in range(nB)]
                    mjobs = [(wg_v, a_) for a_ in range(nA)] + [(wu_v, a_) for a_ in range(nA)]
                    vres = {}
                    mres = {}
                    due = {}
                    for kk in range(len(vjobs)):
                        k = min(len(mjobs) - 1, (kk + 1) * len(mjobs) // len(vjobs) - 1 + LAG)
                        due.setdefault(k, []).append(kk)
                    for k, (wr_, t) in enumerate(mjobs):
                        w = wr_[t]
                        for kk in due.get(k, []):
                            vw, vt = vjobs[kk]
                            res = vpu_tile(vw, vt, 0, D)
                            vres[(id(vw), vt)] = res
                            w = tie_w(w, res)
                        mres[(id(wr_), t)] = jnp.dot(x16, w, preferred_element_type=F32)
                    for vw, vt in vjobs:
                        if (id(vw), vt) not in vres:
                            vres[(id(vw), vt)] = vpu_tile(vw, vt, 0, D)

                    def full(wr_):
                        return _cat([mres[(id(wr_), t)] for t in range(nA)] +
                                    [jnp.broadcast_to(vres[(id(wr_), t)], (16, LT)) for t in range(nA, FT)], 1)
                    gate = full(wg_v)
                    up = full(wu_v)
                    actf = (gate * jax.nn.sigmoid(gate) * up).astype(BF16)
                with scope("t_d"):
                    wait(cp_wd())
                    kA = nA * LT
                    col_v[0:FF - kA, :] = jnp.broadcast_to(actf[0:1, kA:].astype(F32), (LT, FF - kA)).T
                    ys = []
                    vparts = [colsum(wd_v[t, kA:FF, :].astype(F32) * col_v[0:FF - kA, :]) for t in range(DT)]
                    for t in range(DT):
                        w = wd_v[t, 0:kA, :]
                        if t >= 2:
                            w = tie_w(w, vparts[t - 2])
                        ys.append(jnp.dot(actf[:, 0:kA], w, preferred_element_type=F32))
                    y = _cat(ys, 1) + _cat([jnp.broadcast_to(v_, (16, LT)) for v_ in vparts], 1)
                    y = jnp.where(rowid == idx - t0, y, 0.0)
            with scope("t_p"):
                rt = jnp.sum(h2tf * wr_row(), axis=-1, keepdims=True)
                patch_v[...] = (x1_v[trow, :] + modrow(5) * (h2tf + y * jax.nn.sigmoid(rt))).astype(BF16)
                cp_out(0, SQ).wait()
                cp = pltpu.make_async_copy(patch_v, out_hbm.at[trow, :], sems.at[S_PATCH])
                cp.start()
                cp.wait()

    return kernel


def _run(A_x, A_k_cache, A_v_cache, A_wq, A_wo, B_x, B_w_r, B_w_gate, B_w_up, B_w_down, c, w_mod,
        NCQ=8, NCO=8, PROF=False, LASTSPLIT=(160,128,96,64,32,32), QP=7, OP=0, TAILV=0, LAG=0, LSUM=2, MODPOS='o', MT=4, MR=256, MSPLIT=4, flags=None):
    nsem = 8 + NST + 4 * NG + NG * NCQ
    any_spec = pl.BlockSpec(memory_space=pl.ANY)
    out = pl.pallas_call(
        _make_kernel(NCQ, NCO, PROF, LASTSPLIT, QP, OP, TAILV, LAG, LSUM, MODPOS, MT, MR, MSPLIT),
        out_shape=jax.ShapeDtypeStruct((SQ, D), BF16),
        grid=(1,),
        in_specs=[any_spec] * 11,
        out_specs=any_spec,
        scratch_shapes=[
            pltpu.VMEM((SQ, D), BF16),
            pltpu.VMEM((HKV, W, DH), BF16),
            pltpu.VMEM((HKV, W, DH), BF16),
            pltpu.VMEM((HQ, D, LT), BF16),
            pltpu.VMEM((DT, HQ * DH, LT), BF16),
            pltpu.VMEM((DT, LT), BF16),
            pltpu.VMEM((FT, D, LT), BF16),
            pltpu.VMEM((FT, D, LT), BF16),
            pltpu.VMEM((DT, FF, LT), BF16),
            pltpu.VMEM((1, D), BF16),
            pltpu.VMEM((4 * DT, D, LT), BF16),
            pltpu.VMEM((2 * NST, D, SW), BF16),
            pltpu.VMEM((6, DT, 8, LT), F32),
            pltpu.VMEM((D, LT), F32),
            pltpu.VMEM((D + 512, LT), F32),
            pltpu.VMEM((DT, BQ, LT), F32),
            pltpu.VMEM((DT, BQ, LT), BF16),
            pltpu.VMEM((DT, BQ, LT), BF16),
            pltpu.VMEM((REP, BQ, LT), BF16),
            pltpu.VMEM((REP, BQ, LT), BF16),
            pltpu.VMEM((BQ, D), F32),
            pltpu.VMEM((BQ, D), F32),
            pltpu.VMEM((SQ, D), F32),
            pltpu.VMEM((SQ, D), BF16),
            pltpu.VMEM((SQ, D), BF16),
            pltpu.VMEM((16, D), BF16),
            pltpu.VMEM((SQ // PIECE, 8, 128), F32),
            pltpu.VMEM((SQ // PIECE, 8, 128), jnp.int32),
            pltpu.SemaphoreType.DMA((nsem,)),
            pltpu.SemaphoreType.DMA(()),
        ],
        compiler_params=pltpu.CompilerParams(vmem_limit_bytes=110 * 1024 * 1024, flags=flags),
    )(
        A_x.reshape(SQ, D), A_k_cache.reshape(HKV, SK, DH), A_v_cache.reshape(HKV, SK, DH),
        A_wq, A_wo, B_w_r.reshape(DT, LT), B_w_gate, B_w_up, B_w_down, c, w_mod,
    )
    return out.reshape(1, SQ, D)


@jax.jit
def pallas_adaLN_cond__sliding_block_cached__moe_arch_mod__prompt_kernel(
    A_x, A_k_cache, A_v_cache, A_wq, A_wo, B_x, B_w_r, B_w_gate, B_w_up, B_w_down, c, w_mod,
):
    return _run(A_x, A_k_cache, A_v_cache, A_wq, A_wo, B_x, B_w_r, B_w_gate, B_w_up, B_w_down, c, w_mod)
```

```python
import math

import jax
import jax.numpy as jnp
from jax import lax
import jax.experimental.pallas as pl
import jax.experimental.pallas.tpu as pltpu

F32 = jnp.float32
BF16 = jnp.bfloat16

SQ, D = 2048, 1024
HQ, HKV, SK, DH = 32, 4, 2048, 128
W = min(4096, max(256, SK // 4))
REP = HQ // HKV
FF = 3584
EPS = 1e-5
QSCALE = DH ** -0.5 * math.log2(math.e)
GW = REP * DH
NG = HKV
LT = 128
DT = D // LT
FT = FF // LT
BQ = 512
NB = SQ // BQ
CH = BQ // NG
PIECE = 16
NST = 2
SW = D // NST
MSPLIT = 4
LAST_ROWS = (160, 128, 96, 64, 32, 32)
FIRST_WAITS = {0: (0,), 1: (1,), 2: (2, 3), 4: (4, 5, 6, 7)}


def _layernorm(x):
    m = jnp.mean(x, axis=-1, keepdims=True)
    d = x - m
    v = jnp.mean(d * d, axis=-1, keepdims=True)
    return d * lax.rsqrt(v + EPS)


def _recip(l):
    r = pl.reciprocal(l, approx=True)
    return r * (2.0 - l * r)


def _cat(parts, axis):
    return parts[0] if len(parts) == 1 else jnp.concatenate(parts, axis=axis)


def _pieces(n, k):
    t = n // 16
    sizes = [(t // k + (1 if a < t % k else 0)) * 16 for a in range(k)]
    return [(sum(sizes[:a]), sizes[a]) for a in range(k)]


def _tie(tiles, never, dep):
    if dep is None:
        return tiles
    if isinstance(dep, list):
        out = list(tiles)
        for t, a, val in dep:
            lt = out[t]
            parts = [lt[0:a]] if a else []
            parts.append(jnp.where(never, val, lt[a:a + 16]))
            if a + 16 < lt.shape[0]:
                parts.append(lt[a + 16:])
            out[t] = _cat(parts, 0)
        return out
    rows = tiles[0].shape[0]
    ng = dep.shape[0] // 16
    step = rows // (ng * 16) * 16
    out = []
    for t, lt in enumerate(tiles):
        parts = []
        for r in range(ng):
            a = r * step
            parts.append(jnp.where(never, dep[r * 16:(r + 1) * 16, t * LT:(t + 1) * LT], lt[a:a + 16]))
            if step > 16:
                parts.append(lt[a + 16:a + step])
        if ng * step < rows:
            parts.append(lt[ng * step:])
        out.append(_cat(parts, 0))
    return out


def _kernel(x_hbm, k_hbm, v_hbm, wq_hbm, wo_hbm, wr_hbm, wg_hbm, wu_hbm, wd_hbm, c_hbm, wm_hbm,
            out_hbm,
            x_v, k_v, v_v, wq_v, wo_v, wr_v, wg_v, wu_v, wd_v, c_v, wm_v, w01_v,
            mod_v, scol_v, n_v, h_a, h_b, q_v, o_v, acc_a, acc_b, x1_v, h2_v, out_v, patch_v,
            best_v, bidx_v, sems, out_sem):
    h_bufs = (h_a, h_b)
    acc_bufs = (acc_a, acc_b)
    S_C, S_WR, S_WG, S_WU, S_WD, S_PATCH, S_X0, S_XR = range(8)
    S_T = 8
    S_X1 = S_T + NST
    S_KV = S_X1 + NG
    S_WO = S_KV + NG
    S_WM = S_WO + NG
    S_WQ = S_WM + NG

    def start(cps):
        for cp in cps if isinstance(cps, list) else [cps]:
            cp.start()

    def wait(cps):
        for cp in cps if isinstance(cps, list) else [cps]:
            cp.wait()

    def coltile(src, r0, nr, t, dst, sem):
        return pltpu.make_async_copy(src.at[pl.ds(r0, nr), pl.ds(pl.multiple_of(t * LT, LT), LT)], dst, sem)

    def cp_c():
        return pltpu.make_async_copy(c_hbm, c_v, sems.at[S_C])

    def cp_wr():
        return pltpu.make_async_copy(wr_hbm, wr_v, sems.at[S_WR])

    def cp_x0():
        return pltpu.make_async_copy(x_hbm.at[pl.ds(0, BQ), :], x_v.at[pl.ds(0, BQ), :], sems.at[S_X0])

    def cp_x1(g):
        rows = pl.ds(pl.multiple_of(BQ + g * CH, CH), CH)
        return pltpu.make_async_copy(x_hbm.at[rows, :], x_v.at[rows, :], sems.at[S_X1 + g])

    def cp_xrest():
        rows = pl.ds(2 * BQ, SQ - 2 * BQ)
        return pltpu.make_async_copy(x_hbm.at[rows, :], x_v.at[rows, :], sems.at[S_XR])

    def cp_ss(t):
        return [pltpu.make_async_copy(wm_hbm.at[:, pl.ds(pl.multiple_of(j * D + t * SW, SW), SW)],
                                      w01_v.at[j * NST + t], sems.at[S_T + t]) for j in range(2)]

    def cp_kv(g):
        return [pltpu.make_async_copy(k_hbm.at[g, pl.ds(SK - W, W), :], k_v.at[g], sems.at[S_KV + g]),
                pltpu.make_async_copy(v_hbm.at[g, pl.ds(SK - W, W), :], v_v.at[g], sems.at[S_KV + g])]

    def cp_wq(g, j):
        return coltile(wq_hbm, 0, D, g * REP + j, wq_v.at[g * REP + j], sems.at[S_WQ + g * REP + j])

    def cp_wo(g):
        r0 = pl.multiple_of(g * GW, GW)
        return [coltile(wo_hbm, r0, GW, t, wo_v.at[t, pl.ds(r0, GW), :], sems.at[S_WO + g]) for t in range(DT)]

    def cp_wm(g):
        return [coltile(wm_hbm, 0, D, (2 + g) * DT + t, wm_v.at[g * DT + t], sems.at[S_WM + g])
                for t in range(DT)]

    def cp_wg():
        return [coltile(wg_hbm, 0, D, t, wg_v.at[t], sems.at[S_WG]) for t in range(FT)]

    def cp_wu():
        return [coltile(wu_hbm, 0, D, t, wu_v.at[t], sems.at[S_WU]) for t in range(FT)]

    def cp_wd():
        return [coltile(wd_hbm, 0, FF, t, wd_v.at[t], sems.at[S_WD]) for t in range(DT)]

    def cp_out(r0, n):
        return pltpu.make_async_copy(out_v.at[pl.ds(r0, n), :], out_hbm.at[pl.ds(r0, n), :], out_sem)

    def modrow(j):
        return _cat([mod_v[j, t, 0:1, :] for t in range(DT)], 1)

    def wr_row():
        w = wr_v[...].astype(F32)
        return _cat([w[t:t + 1, :] for t in range(DT)], 1)

    def silu_c():
        cf = c_v[...].astype(F32)
        return (cf * jax.nn.sigmoid(cf)).astype(BF16)

    def ln1(r0, n, slot, o0):
        xf = x_v[pl.ds(r0, n), :].astype(F32)
        h = (_layernorm(xf) * (1.0 + modrow(1)) + modrow(0)).astype(BF16)
        for t in range(DT):
            h_bufs[slot][t, pl.ds(o0, n), :] = h[:, t * LT:(t + 1) * LT]
        return h

    def epilogue(r0, n, attn):
        rows = pl.ds(r0, n)
        x1 = x_v[rows, :].astype(F32) + modrow(2) * attn
        h2 = (_layernorm(x1) * (1.0 + modrow(4)) + modrow(3)).astype(BF16)
        h2f = h2.astype(F32)
        x1_v[rows, :] = x1
        h2_v[rows, :] = h2
        out = (x1 + modrow(5) * h2f).astype(BF16)
        out_v[rows, :] = out
        r = jnp.sum(h2f * wr_row(), axis=-1, keepdims=True)
        r = r.astype(BF16).astype(F32)
        r3 = jnp.broadcast_to(r, (n, LT)).reshape(n // 8, 8, LT)
        sub = lax.broadcasted_iota(jnp.int32, (8, LT), 0) + r0
        best = r3[0]
        bidx = sub
        for t in range(1, n // 8):
            upd = r3[t] > best
            best = jnp.where(upd, r3[t], best)
            bidx = jnp.where(upd, sub + t * 8, bidx)
        best_v[r0 // PIECE] = best
        bidx_v[r0 // PIECE] = bidx
        return out

    def mod_tile(j, t):
        kq = D // MSPLIT
        deps = []
        acc8 = None
        for k_ in range(MSPLIT):
            rs = slice(k_ * kq, (k_ + 1) * kq)
            p8 = (wm_v[(j - 2) * DT + t, rs, :].astype(F32) * scol_v[rs, :]).reshape(kq // 8, 8, LT).sum(axis=0)
            acc8 = p8 if acc8 is None else acc8 + p8
            if k_ + 1 < MSPLIT:
                pos = (k_ + 1) * 64 // MSPLIT
                deps.append(((0 if pos < 32 else 4) + k_ % 4, (pos % 32) * 16,
                             jnp.concatenate([p8, p8], axis=0).astype(BF16)))
        y = jnp.sum(acc8, axis=0, keepdims=True)
        mod_v[j, t] = jnp.broadcast_to(y, (8, LT))
        deps.append((REP - 1, BQ - 16, jnp.broadcast_to(y.astype(BF16), (16, LT))))
        return deps

    def q_and_attention(slot, g, never, qdeps, pre_q):
        hb = h_bufs[slot]
        for j in range(REP):
            if pre_q is not None:
                pre_q(j)
            dep = qdeps[j]() if qdeps[j] else None
            lhs = _cat(_tie([hb[t] for t in range(DT)], never, dep), 1)
            q = jnp.dot(lhs, wq_v[g * REP + j], preferred_element_type=F32)
            q_v[j] = (q * QSCALE).astype(BF16)
        for hh in range(REP):
            s = lax.dot_general(q_v[hh], k_v[g], (((1,), (1,)), ((), ())), preferred_element_type=F32)
            m = jnp.max(s, axis=-1, keepdims=True)
            p = jnp.exp2(s - m).astype(BF16)
            l = jnp.sum(p.astype(F32), axis=-1, keepdims=True)
            o = jnp.dot(p, v_v[g], preferred_element_type=F32)
            o_v[hh] = (o * _recip(l)).astype(BF16)

    def out_projection(slot, g, never, odeps):
        acc = acc_bufs[slot]
        g0 = pl.multiple_of(g * GW, GW)
        for j in range(DT):
            dep = odeps[j]() if odeps[j] else None
            lhs = _cat(_tie([o_v[t] for t in range(REP)], never, dep), 1)
            d = jnp.dot(lhs, wo_v[j, pl.ds(g0, GW), :], preferred_element_type=F32)
            cs = slice(j * LT, (j + 1) * LT)
            acc[:, cs] = jnp.where(g == 0, 0.0, acc[:, cs]) + d

    def last_out_projection(slot, g, never):
        acc = acc_bufs[slot]
        g0 = pl.multiple_of(g * GW, GW)
        dep = None
        r0 = 0
        for rc in LAST_ROWS:
            rows = slice(r0, r0 + rc)
            if dep is not None and dep.shape[0] > rc:
                parts = [dep[a:a + rc] for a in range(0, dep.shape[0] - rc + 1, rc)]
                if dep.shape[0] % rc:
                    parts.append(dep[dep.shape[0] - rc:])
                dep = parts[0]
                for p_ in parts[1:]:
                    dep = jnp.where(never, p_, dep)
            lhs = _cat(_tie([o_v[t, rows, :] for t in range(REP)], never, dep), 1)
            w = _cat([wo_v[n, pl.ds(g0, GW), :] for n in range(DT)], 1)
            attn = acc[rows, :] + jnp.dot(lhs, w, preferred_element_type=F32)
            dep = epilogue((NB - 1) * BQ + r0, rc, attn)
            r0 += rc

    start(cp_c())
    start(cp_x0())
    for t in range(NST):
        start(cp_ss(t))
    for j in range(REP):
        start(cp_wq(0, j))
        if j == 0:
            start(cp_x1(0))
        if j == 1:
            start(cp_kv(0))

    best_v[...] = jnp.full(best_v.shape, -jnp.inf, F32)
    bidx_v[...] = jnp.zeros(bidx_v.shape, jnp.int32)

    wait(cp_c())
    wait(cp_x0())

    def ln_body(r, carry):
        r0 = pl.multiple_of(r * CH, CH)
        n = _layernorm(x_v[pl.ds(r0, CH), :].astype(F32))
        for t in range(DT):
            n_v[t, pl.ds(r0, CH), :] = n[:, t * LT:(t + 1) * LT]
        return carry
    lax.fori_loop(0, BQ // CH, ln_body, 0)
    start(cp_wo(0))
    start(cp_wm(0))
    start(cp_wr())
    scol_v[...] = jnp.broadcast_to(silu_c().astype(F32), (LT, D)).T

    def shift_scale_body(t, carry):
        wait(cp_ss(t))
        sc = jnp.broadcast_to(silu_c(), (16, D))
        sa = jnp.dot(sc, w01_v[t], preferred_element_type=F32)[0:8, :]
        ca = jnp.dot(sc, w01_v[NST + t], preferred_element_type=F32)[0:8, :]
        for u in range(SW // LT):
            tt = t * (SW // LT) + u
            cs = slice(u * LT, (u + 1) * LT)
            mod_v[0, tt] = sa[:, cs]
            mod_v[1, tt] = ca[:, cs]
            h_a[tt] = (n_v[tt] * (1.0 + ca[0:1, cs]) + sa[0:1, cs]).astype(BF16)
        return carry
    lax.fori_loop(0, NST, shift_scale_body, 0)

    for i in range(NB):
        slot = i % 2

        def unit(g, carry, i=i, slot=slot, first=False, last=False):
            never = g < 0

            def side(o, n):
                def f():
                    o0 = pl.multiple_of(g * CH + o, 16)
                    e = None
                    if i > 0:
                        e = epilogue(pl.multiple_of((i - 1) * BQ + o0, 16), n,
                                     acc_bufs[1 - slot][pl.ds(o0, n), :])
                    if i + 1 < NB:
                        hv = ln1(pl.multiple_of((i + 1) * BQ + o0, 16), n, 1 - slot, o0)
                        e = hv if e is None else jnp.where(never, hv, e)
                    return e
                return f

            qdeps = [None] + [side(o, n) for o, n in _pieces(CH, REP - 1)]
            odeps = [None] * DT
            pre_q = None
            if i == 0:
                @pl.when(g + 1 < NG)
                def _():
                    for j in range(REP):
                        start(cp_wq(g + 1, j))
                    start(cp_kv(g + 1))
                    start(cp_x1(g + 1))
                    start(cp_wo(g + 1))
                    start(cp_wm(g + 1))

                @pl.when(g == NG - 2)
                def _():
                    start(cp_xrest())

                if first:
                    def pre_q(j):
                        for jj in FIRST_WAITS.get(j, ()):
                            wait(cp_wq(g, jj))
                        if j == 1:
                            wait(cp_x1(g))
                        if j == 4:
                            wait(cp_kv(g))
                else:
                    wait(cp_x1(g))
                    for j in range(REP):
                        wait(cp_wq(g, j))
                    wait(cp_kv(g))
                    wait(cp_wo(g))
                    wait(cp_wm(g))
                odeps = [(lambda t=t: mod_tile(2 + g, t)) for t in range(DT)]

            q_and_attention(slot, g, never, qdeps, pre_q)
            if first:
                wait(cp_wo(g))
                wait(cp_wm(g))
            if last:
                last_out_projection(slot, g, never)
            else:
                out_projection(slot, g, never, odeps)
            if i > 0:
                cp_out(pl.multiple_of((i - 1) * BQ + g * CH, CH), CH).start()
            return carry

        if i == 0:
            unit(pl.program_id(0), 0, first=True)
            lax.fori_loop(1, NG, unit, 0)
            wait(cp_wr())
            wait(cp_xrest())
            start(cp_wg())
            start(cp_wu())
            start(cp_wd())
        elif i == NB - 1:
            lax.fori_loop(0, NG - 1, unit, 0)
            unit(pl.program_id(0) + (NG - 1), 0, last=True)
        else:
            lax.fori_loop(0, NG, unit, 0)

    cp_out((NB - 1) * BQ, BQ).start()

    ent = [(best_v[t], bidx_v[t]) for t in range(SQ // PIECE)]
    while len(ent) > 1:
        nxt = []
        for t in range(0, len(ent), 2):
            (b0, i0), (b1, i1) = ent[t], ent[t + 1]
            upd = b1 > b0
            nxt.append((jnp.where(upd, b1, b0), jnp.where(upd, i1, i0)))
        ent = nxt
    best, bidx = ent[0]
    mx = jnp.max(best, axis=0, keepdims=True)
    idx = jnp.clip(jnp.min(jnp.where(best == mx, bidx, SQ)), 0, SQ - 1)
    t0 = pl.multiple_of((idx // 16) * 16, 16)
    trow = pl.ds(t0, 16)
    h2t = h2_v[trow, :].astype(F32)
    rowid = lax.broadcasted_iota(jnp.int32, (16, D), 0)
    xsel = jnp.where(rowid == idx - t0, h2t, 0.0).astype(BF16)
    wait(cp_wg())
    gate = jnp.dot(xsel, _cat([wg_v[t] for t in range(FT)], 1), preferred_element_type=F32)
    wait(cp_wu())
    up = jnp.dot(xsel, _cat([wu_v[t] for t in range(FT)], 1), preferred_element_type=F32)
    act = (gate * jax.nn.sigmoid(gate) * up).astype(BF16)
    wait(cp_wd())
    y = jnp.dot(act, _cat([wd_v[t] for t in range(DT)], 1), preferred_element_type=F32)
    rt = jnp.sum(h2t * wr_row(), axis=-1, keepdims=True)
    patch_v[...] = (x1_v[trow, :] + modrow(5) * (h2t + y * jax.nn.sigmoid(rt))).astype(BF16)
    cp_out(0, SQ).wait()
    cp = pltpu.make_async_copy(patch_v, out_hbm.at[trow, :], sems.at[S_PATCH])
    cp.start()
    cp.wait()


@jax.jit
def pallas_adaLN_cond__sliding_block_cached__moe_arch_mod__prompt_kernel(
    A_x, A_k_cache, A_v_cache, A_wq, A_wo, B_x, B_w_r, B_w_gate, B_w_up, B_w_down, c, w_mod,
):
    del B_x
    any_spec = pl.BlockSpec(memory_space=pl.ANY)
    out = pl.pallas_call(
        _kernel,
        out_shape=jax.ShapeDtypeStruct((SQ, D), BF16),
        grid=(1,),
        in_specs=[any_spec] * 11,
        out_specs=any_spec,
        scratch_shapes=[
            pltpu.VMEM((SQ, D), BF16),
            pltpu.VMEM((HKV, W, DH), BF16),
            pltpu.VMEM((HKV, W, DH), BF16),
            pltpu.VMEM((HQ, D, LT), BF16),
            pltpu.VMEM((DT, HQ * DH, LT), BF16),
            pltpu.VMEM((DT, LT), BF16),
            pltpu.VMEM((FT, D, LT), BF16),
            pltpu.VMEM((FT, D, LT), BF16),
            pltpu.VMEM((DT, FF, LT), BF16),
            pltpu.VMEM((1, D), BF16),
            pltpu.VMEM((4 * DT, D, LT), BF16),
            pltpu.VMEM((2 * NST, D, SW), BF16),
            pltpu.VMEM((6, DT, 8, LT), F32),
            pltpu.VMEM((D, LT), F32),
            pltpu.VMEM((DT, BQ, LT), F32),
            pltpu.VMEM((DT, BQ, LT), BF16),
            pltpu.VMEM((DT, BQ, LT), BF16),
            pltpu.VMEM((REP, BQ, LT), BF16),
            pltpu.VMEM((REP, BQ, LT), BF16),
            pltpu.VMEM((BQ, D), F32),
            pltpu.VMEM((BQ, D), F32),
            pltpu.VMEM((SQ, D), F32),
            pltpu.VMEM((SQ, D), BF16),
            pltpu.VMEM((SQ, D), BF16),
            pltpu.VMEM((16, D), BF16),
            pltpu.VMEM((SQ // PIECE, 8, LT), F32),
            pltpu.VMEM((SQ // PIECE, 8, LT), jnp.int32),
            pltpu.SemaphoreType.DMA((8 + NST + 4 * NG + HQ,)),
            pltpu.SemaphoreType.DMA(()),
        ],
        compiler_params=pltpu.CompilerParams(vmem_limit_bytes=110 * 1024 * 1024),
    )(
        A_x.reshape(SQ, D), A_k_cache.reshape(HKV, SK, DH), A_v_cache.reshape(HKV, SK, DH),
        A_wq, A_wo, B_w_r.reshape(DT, LT), B_w_gate, B_w_up, B_w_down, c, w_mod,
    )
    return out.reshape(1, SQ, D)
```
